```python
import os as _os
_os.environ.setdefault("JAX_PLATFORMS", "cpu")
import jax
import jax.numpy as jnp

def _softmax(x, axis=-1):
    return jax.nn.softmax(x, axis=axis)
def _gelu(x):
    return jax.nn.gelu(x, approximate=True)
def _silu(x):
    return jax.nn.silu(x)
def _sigmoid(x):
    return jax.nn.sigmoid(x)
def _layernorm(x, axis=-1, eps=1e-5):
    m = jnp.mean(x, axis=axis, keepdims=True)
    v = jnp.var(x, axis=axis, keepdims=True)
    return (x - m) / jnp.sqrt(v + eps)
def _scatter_add(tgt, idx, src, axis=0):
    return tgt.at[idx].add(src)
def _segment_sum(src, seg, n):
    return jax.ops.segment_sum(src, seg, n)
class _Rng:
    def __init__(self, key):
        self._k = key
    def _next(self):
        self._k, sub = jax.random.split(self._k)
        return sub
    def normal(self, shape):
        return jax.random.normal(self._next(), shape, dtype=jnp.bfloat16)
    def randint(self, lo, hi, shape):
        return jax.random.randint(self._next(), shape, lo, hi, dtype=jnp.int32)
    def uniform(self, shape, lo=0.0, hi=1.0):
        return jax.random.uniform(self._next(), shape, jnp.bfloat16, lo, hi)
    def permutation(self, n):
        return jax.random.permutation(self._next(), n)


kernel_name = 'standalone__gqa_block_cached__near_ridge'

def setup_inputs():
    _rng = _Rng(jax.random.key(int.from_bytes(__import__("os").urandom(4), "little")))
    _w = (lambda a: (lambda t: t.astype(jnp.bfloat16) if jnp.issubdtype(t.dtype, jnp.floating) else t)(jnp.asarray(a)))
    B, Sq, D = 8, 64, 512
    Hq, Hkv, Sk, Dh = 32, 8, 64, 128
    assert Hq % Hkv == 0, (Hq, Hkv)
    return {
        "x": _w((lambda *s: _rng.normal(s) * 0.8)(B, Sq, D)),
        "k_cache": _w((lambda *s: _rng.normal(s) * 0.8)(B, Hkv, Sk, Dh)),
        "v_cache": _w((lambda *s: _rng.normal(s) * 0.05)(B, Hkv, Sk, Dh)),
        "wq": _w((lambda *s: _rng.normal(s) * 0.8)(D, Hq * Dh) * (D ** -0.5)),
        "wo": _w((lambda *s: _rng.normal(s) * 0.05)(Hq * Dh, D) * ((Hq * Dh) ** -0.5)),
    }

def reference(x, k_cache, v_cache, wq, wo):
    B, Sq, D = x.shape
    Hq, Dh = 32, 128
    Hkv = k_cache.shape[1]
    rep = Hq // Hkv
    q = (lambda x, *d: x.transpose(*d))((x @ wq).reshape(B, Sq, Hq, Dh), 0, 2, 1, 3)
    k = jnp.repeat(k_cache, rep, axis=1)
    v = jnp.repeat(v_cache, rep, axis=1)
    scores = jnp.einsum("bhqd,bhkd->bhqk", q, k) * (Dh ** -0.5)
    p = _softmax(scores, axis=-1)
    o = jnp.einsum("bhqk,bhkd->bhqd", p, v)
    return (lambda x, *d: x.transpose(*d))(o, 0, 2, 1, 3).reshape(B, Sq, Hq * Dh) @ wo
```

```python
import math
import jax
import jax.numpy as jnp
from jax import lax
import jax.experimental.pallas as pl
import jax.experimental.pallas.tpu as pltpu

BARRIERS = '1,2,4'
QK0 = '128,128,256'
OCH = '128,128,128,128'


@jax.jit
def pallas_standalone__gqa_block_cached__near_ridge_kernel(x, k_cache, v_cache, wq, wo):
    B, Sq, D = x.shape
    _, Hkv, Sk, Dh = k_cache.shape
    Hq = wq.shape[1] // Dh
    rep = Hq // Hkv
    GW = rep * Dh
    M = B * Sq
    scale = float(Dh) ** -0.5
    c2 = scale * math.log2(math.e)
    x2 = x.reshape(M, D)
    bf16 = jnp.bfloat16
    f32 = jnp.float32
    NT = (((1,), (1,)), ((), ()))

    kch = [int(s) for s in QK0.split(',')]
    assert sum(kch) == D
    koff = [sum(kch[:i]) for i in range(len(kch))]
    nk0 = len(kch)
    och = [int(s) for s in OCH.split(',')]
    assert sum(och) == M and all(c % Sq == 0 for c in och)
    ooff = [sum(och[:i]) for i in range(len(och))]
    bsteps = [int(s) for s in BARRIERS.split(',')]
    assert bsteps[0] == 1
    cover = {g: max(b for b in bsteps if b <= g) for g in range(1, Hkv)}

    bar_names = [('q0', p) for p in range(nk0)] + [('s0',), ('p0',)] + [('step', b) for b in bsteps]
    bar_idx = {n: i for i, n in enumerate(bar_names)}
    n_bar = len(bar_names)

    def bar_of(name):
        kind, i = name
        if kind in ('x', 'wq0'):
            return bar_idx[('q0', i)]
        if kind == 'k':
            g_use = i - 1
            if i == 0:
                return bar_idx[('s0',)]
        elif kind == 'wq':
            g_use = i - 1
            if g_use == 0:
                return bar_idx[('s0',)]
        else:
            g_use = i
        if g_use == 0:
            return bar_idx[('p0',)]
        return bar_idx[('step', cover[g_use])]

    fifo = []
    for p in range(nk0):
        fifo += [('x', p), ('wq0', p)]
    fifo.append(('k', 0))
    for g in range(Hkv):
        if g + 1 < Hkv:
            fifo.append(('wq', g + 1))
        fifo += [('v', g), ('wo', g)]
        if g + 1 < Hkv:
            fifo.append(('k', g + 1))

    def kernel(x_hbm, wq_hbm, k_hbm, v_hbm, wo_hbm, out_hbm,
               x_v, wq_v, wo_v, k_v, v_v, q0, q1, o_s, acc, out_v, s_scr,
               sem_in, sem_out):
        qs = (q0, q1)

        def cp(name):
            kind, i = name
            sem = sem_in.at[bar_of(name)]
            if kind == 'x':
                return pltpu.make_async_copy(x_hbm.at[:, pl.ds(koff[i], kch[i])],
                                             x_v.at[:, pl.ds(koff[i], kch[i])], sem)
            if kind == 'wq0':
                return pltpu.make_async_copy(wq_hbm.at[pl.ds(koff[i], kch[i]), pl.ds(0, GW)],
                                             wq_v.at[0, pl.ds(koff[i], kch[i]), :], sem)
            if kind == 'wq':
                return pltpu.make_async_copy(wq_hbm.at[:, pl.ds(i * GW, GW)], wq_v.at[i], sem)
            if kind == 'wo':
                return pltpu.make_async_copy(wo_hbm.at[pl.ds(i * GW, GW), :], wo_v.at[i], sem)
            if kind == 'k':
                return pltpu.make_async_copy(k_hbm.at[:, i], k_v.at[i], sem)
            if kind == 'v':
                return pltpu.make_async_copy(v_hbm.at[:, i], v_v.at[i], sem)
            raise ValueError(name)

        def barrier(bname):
            bi = bar_idx[bname]
            for name in fifo:
                if bar_of(name) == bi:
                    cp(name).wait()

        def qproj(g):
            q = jnp.dot(x_v[...], wq_v[g], preferred_element_type=f32)
            qs[g % 2][...] = q.astype(bf16)

        def scores(g):
            q_ref = qs[g % 2]
            for b in range(B):
                qb = q_ref[b * Sq:(b + 1) * Sq, :]
                qstack = jnp.concatenate([qb[:, h * Dh:(h + 1) * Dh] for h in range(rep)], axis=0)
                s_scr[b] = lax.dot_general(k_v[g, b], qstack, NT, preferred_element_type=f32)

        def softmax_pv(g, batches):
            for b in batches:
                st = s_scr[b]
                m = jnp.max(st, axis=0, keepdims=True)
                pt = jnp.exp2((st - m) * c2)
                l = jnp.sum(pt, axis=0, keepdims=True)
                pt = pt / l
                o = jnp.dot(pt.T.astype(bf16), v_v[g, b], preferred_element_type=f32)
                ob = jnp.concatenate([o[h * Sq:(h + 1) * Sq] for h in range(rep)], axis=1)
                o_s[b * Sq:(b + 1) * Sq, :] = ob.astype(bf16)

        def outproj(g):
            contrib = jnp.dot(o_s[...], wo_v[g], preferred_element_type=f32)
            if g == 0:
                acc[...] = contrib
            else:
                acc[...] += contrib

        def out_copy(c):
            return pltpu.make_async_copy(out_v.at[pl.ds(ooff[c], och[c]), :],
                                         out_hbm.at[pl.ds(ooff[c], och[c]), :], sem_out.at[0])

        for name in fifo:
            cp(name).start()

        for p in range(nk0):
            barrier(('q0', p))
            part = jnp.dot(x_v[:, koff[p]:koff[p] + kch[p]], wq_v[0, koff[p]:koff[p] + kch[p], :],
                           preferred_element_type=f32)
            if nk0 == 1:
                q0[...] = part.astype(bf16)
            elif p == 0:
                acc[...] = part
            elif p < nk0 - 1:
                acc[...] += part
            else:
                q0[...] = (acc[...] + part).astype(bf16)
        barrier(('s0',))
        scores(0)

        for g in range(Hkv):
            last = g == Hkv - 1
            if g in bsteps:
                barrier(('step', g))
            if not last:
                qproj(g + 1)
                if g == 0:
                    barrier(('p0',))
                softmax_pv(g, range(B))
                scores(g + 1)
                outproj(g)
            else:
                for c in range(len(och)):
                    softmax_pv(g, range(ooff[c] // Sq, (ooff[c] + och[c]) // Sq))
                    rs = slice(ooff[c], ooff[c] + och[c])
                    contrib = jnp.dot(o_s[rs, :], wo_v[g], preferred_element_type=f32)
                    out_v[rs, :] = (acc[rs, :] + contrib).astype(out_v.dtype)
                    out_copy(c).start()
                for c in range(len(och)):
                    out_copy(c).wait()

    out = pl.pallas_call(
        kernel,
        in_specs=[pl.BlockSpec(memory_space=pl.ANY)] * 5,
        out_specs=pl.BlockSpec(memory_space=pl.ANY),
        out_shape=jax.ShapeDtypeStruct((M, D), x.dtype),
        scratch_shapes=[
            pltpu.VMEM((M, D), bf16),
            pltpu.VMEM((Hkv, D, GW), bf16),
            pltpu.VMEM((Hkv, GW, D), bf16),
            pltpu.VMEM((Hkv, B, Sk, Dh), bf16),
            pltpu.VMEM((Hkv, B, Sk, Dh), bf16),
            pltpu.VMEM((M, GW), bf16),
            pltpu.VMEM((M, GW), bf16),
            pltpu.VMEM((M, GW), bf16),
            pltpu.VMEM((M, D), f32),
            pltpu.VMEM((M, D), bf16),
            pltpu.VMEM((B, Sk, rep * Sq), f32),
            pltpu.SemaphoreType.DMA((n_bar,)),
            pltpu.SemaphoreType.DMA((1,)),
        ],
        compiler_params=pltpu.CompilerParams(
            vmem_limit_bytes=100 * 1024 * 1024,
        ),
    )(x2, wq, k_cache, v_cache, wo)
    return out.reshape(B, Sq, D)
```
